```python
import os as _os
_os.environ.setdefault("JAX_PLATFORMS", "cpu")
import jax
import jax.numpy as jnp

def _softmax(x, axis=-1):
    return jax.nn.softmax(x, axis=axis)
def _gelu(x):
    return jax.nn.gelu(x, approximate=True)
def _silu(x):
    return jax.nn.silu(x)
def _sigmoid(x):
    return jax.nn.sigmoid(x)
def _layernorm(x, axis=-1, eps=1e-5):
    m = jnp.mean(x, axis=axis, keepdims=True)
    v = jnp.var(x, axis=axis, keepdims=True)
    return (x - m) / jnp.sqrt(v + eps)
def _scatter_add(tgt, idx, src, axis=0):
    return tgt.at[idx].add(src)
def _segment_sum(src, seg, n):
    return jax.ops.segment_sum(src, seg, n)
class _Rng:
    def __init__(self, key):
        self._k = key
    def _next(self):
        self._k, sub = jax.random.split(self._k)
        return sub
    def normal(self, shape):
        return jax.random.normal(self._next(), shape, dtype=jnp.bfloat16)
    def randint(self, lo, hi, shape):
        return jax.random.randint(self._next(), shape, lo, hi, dtype=jnp.int32)
    def uniform(self, shape, lo=0.0, hi=1.0):
        return jax.random.uniform(self._next(), shape, jnp.bfloat16, lo, hi)
    def permutation(self, n):
        return jax.random.permutation(self._next(), n)


kernel_name = 'sequential_preLN__sliding_local_dilated__dense_activation_relu__prompt'

def setup_inputs():
    _rng = _Rng(jax.random.key(int.from_bytes(__import__("os").urandom(4), "little")))
    _w = (lambda a: (lambda t: t.astype(jnp.bfloat16) if jnp.issubdtype(t.dtype, jnp.floating) else t)(jnp.asarray(a)))
    def _A_setup():
        B, S, D = 1, 2048, 1024
        return {
            "x": _w((lambda *s: _rng.normal(s) * 0.05)(B, S, D)),
            "wqkv": _w((lambda *s: _rng.normal(s) * 0.05)(D, 3 * D)),
            "wo": _w((lambda *s: _rng.normal(s) * 0.05)(D, D)),
        }
    _A_in = _A_setup()

    def _B_setup():
        B, S, D, Dff = 1, 2048, 1024, 3584
        return {
            "x": _w((lambda *s: _rng.normal(s) * 0.05)(B, S, D)),
            "w1": _w((lambda *s: _rng.normal(s) * 0.05)(D, Dff)),
            "w2": _w((lambda *s: _rng.normal(s) * 0.05)(Dff, D)),
        }
    _B_in = _B_setup()

    return {
        "A_x": _A_in["x"],
        "A_wqkv": _A_in["wqkv"],
        "A_wo": _A_in["wo"],
        "B_x": _B_in["x"],
        "B_w1": _B_in["w1"],
        "B_w2": _B_in["w2"],
    }

def reference(A_x, A_wqkv, A_wo, B_x, B_w1, B_w2):
    def _A_ref(x, wqkv, wo):
        B, S, D = x.shape
        H = 32; Dh = D // H
        W, dil = 8, 2
        qkv = (lambda x, *d: x.transpose(*d))((x @ wqkv).reshape(B, S, 3, H, Dh), 2, 0, 3, 1, 4)
        q, k, v = qkv[0], qkv[1], qkv[2]
        scale = Dh ** -0.5
        pos = jnp.arange(S)
        off = jnp.arange(W) * dil
        idx = pos[:, None] - off[None, :]
        mask = idx >= 0
        idx_c = jnp.where(mask, idx, 0).reshape(-1)
        kg = k[:, :, idx_c, :].reshape(B, H, S, W, Dh)
        vg = v[:, :, idx_c, :].reshape(B, H, S, W, Dh)
        logits = jnp.einsum("bhsd,bhswd->bhsw", q, kg) * scale
        logits = jnp.where(mask[None, None, :, :], logits, -1e9)
        attn = _softmax(logits, axis=-1)
        o = jnp.einsum("bhsw,bhswd->bhsd", attn, vg)
        return (lambda x, *d: x.transpose(*d))(o, 0, 2, 1, 3).reshape(B, S, D) @ wo

    def _B_ref(x, w1, w2):
        h = jnp.einsum("bsd,df->bsf", x, w1)
        zero = jnp.zeros_like(h)
        h = jnp.maximum(h, zero)
        return jnp.einsum("bsf,fd->bsd", h, w2)

    x = A_x
    h = x + _A_ref(_layernorm(x, axis=-1), A_wqkv, A_wo)
    h2 = h + _B_ref(_layernorm(h, axis=-1), B_w1, B_w2)
    return h2
```

```python
import functools

import jax
import jax.numpy as jnp
import jax.experimental.pallas as pl
import jax.experimental.pallas.tpu as pltpu

S, D, DFF = 2048, 1024, 3584
H, DH, W = 32, 32, 8
U32, F32, BF16 = jnp.uint32, jnp.float32, jnp.bfloat16
HAL = 16
LOG2E = 1.4426950408889634


def lane_iota(shape):
    return jax.lax.broadcasted_iota(jnp.int32, shape, len(shape) - 1)


def perm_net(tiles):
    lane = lane_iota(tiles[0].shape)
    for b in range(3):
        d = 1 << b
        sh = 4 * d
        m = (lane & sh) == 0
        new = list(tiles)
        for t in range(8):
            if t & d == 0:
                a, bb = tiles[t], tiles[t + d]
                new[t] = jnp.where(m, a, pltpu.roll(bb, sh, 1))
                new[t + d] = jnp.where(m, pltpu.roll(a, 128 - sh, 1), bb)
        tiles = new
    return tiles


def allreduce4(x):
    lane = lane_iota(x.shape)
    y = x + jnp.take_along_axis(x, lane ^ 1, axis=1)
    return y + jnp.take_along_axis(y, lane ^ 2, axis=1)


def ln(x):
    m = jnp.mean(x, axis=-1, keepdims=True)
    xc = x - m
    v = jnp.mean(xc * xc, axis=-1, keepdims=True)
    return xc * jax.lax.rsqrt(v + 1e-5)


TM = 256
M = TM // 2
NT = S // TM
FCH = 512
NF = DFF // FCH
NATT = 4
WO_POS = 4
C2 = DH ** -0.5 * LOG2E


def _kernel(x_ref, wqkv_hbm, wo_hbm, w1_hbm, w2_hbm, o_ref, wqkv_ref, wo_ref, w1_ref, w2_ref, sems, q_all, k_all, v_all, oa_all):
    step = pl.program_id(0)
    cq = [pltpu.make_async_copy(wqkv_hbm.at[:, pl.ds(c * D, D)], wqkv_ref.at[:, pl.ds(c * D, D)], sems.at[c]) for c in range(3)]
    cr = [pltpu.make_async_copy(wo_hbm, wo_ref, sems.at[3]),
          pltpu.make_async_copy(w1_hbm, w1_ref, sems.at[4]),
          pltpu.make_async_copy(w2_hbm, w2_ref, sems.at[5])]

    @pl.when(step == 0)
    def _():
        for c in cq + cr:
            c.start()
        k_all[:, 0:HAL, :] = jnp.zeros((8, HAL, 128), F32)
        v_all[:, 0:HAL, :] = jnp.zeros((8, HAL, 128), F32)
        for c in cq:
            c.wait()

    @pl.when(step == NT)
    def _():
        for c in cr:
            c.wait()

    tile = jnp.where(step < NT, step, step - NT)
    row0 = pl.multiple_of(tile * TM, TM)
    q_s = q_all.at[:, pl.ds(row0, TM), :]
    k_s = k_all.at[:, pl.ds(row0, TM + HAL), :]
    v_s = v_all.at[:, pl.ds(row0, TM + HAL), :]
    oa_s = oa_all.at[pl.ds(pl.multiple_of(tile * (M // 2), M // 2), M // 2), :]

    def qkv_part(xn, c, r0):
        dst, off = ((q_s, 0), (k_s, HAL), (v_s, HAL))[c]
        y = jnp.dot(xn, wqkv_ref[:, c * D:(c + 1) * D], preferred_element_type=F32)
        for r in range(M // 8):
            tiles = perm_net([y[8 * r:8 * r + 8, t * 128:(t + 1) * 128] for t in range(8)])
            for j in range(8):
                dst[j, off + r0 + 8 * r:off + r0 + 8 * r + 8, :] = tiles[j]

    def att8(r):
        q = [q_s[j, r:r + 8, :] for j in range(8)]
        t = []
        for w in range(W):
            acc = None
            for j in range(8):
                p = q[j] * k_s[j, HAL + r - 2 * w:HAL + r - 2 * w + 8, :]
                acc = p if acc is None else acc + p
            l = allreduce4(acc) * C2
            if 2 * w > r:
                pos = row0 + r + jax.lax.broadcasted_iota(jnp.int32, (8, 128), 0)
                l = jnp.where(pos >= 2 * w, l, -1e9 * LOG2E)
            t.append(l)
        m = functools.reduce(jnp.maximum, t)
        e = [jnp.exp2(x - m) for x in t]
        inv = 1.0 / functools.reduce(jnp.add, e)
        a = [x * inv for x in e]
        outs = []
        for j in range(8):
            acc = None
            for w in range(W):
                p = a[w] * v_s[j, HAL + r - 2 * w:HAL + r - 2 * w + 8, :]
                acc = p if acc is None else acc + p
            outs.append(acc)
        return outs

    def att16(r):
        lo, hi = att8(r), att8(r + 8)
        pk = [pltpu.bitcast(jnp.concatenate([lo[j], hi[j]], axis=0).astype(BF16), U32) for j in range(8)]
        return jnp.concatenate(perm_net(pk), axis=1)

    @pl.when(step < NT)
    def _():
        xs = [x_ref[i * M:(i + 1) * M, :].astype(F32) for i in range(2)]
        xn = [ln(x).astype(BF16) for x in xs]
        for c in range(3):
            qkv_part(xn[0], c, 0)
        for c in range(3):
            qkv_part(xn[1], c, M)
            for g in range(c * (M // 16) // 3, (c + 1) * (M // 16) // 3):
                oa_s[8 * g:8 * g + 8, :] = att16(16 * g)

    @pl.when(step >= NT)
    def _():
        def wo_part(i, o):
            h = x_ref[i * M:(i + 1) * M, :].astype(F32) + jnp.dot(o, wo_ref[...], preferred_element_type=F32)
            return h, ln(h).astype(BF16)

        def ffn_chunk(hn, c, acc):
            a = jnp.dot(hn, w1_ref[:, c * FCH:(c + 1) * FCH], preferred_element_type=F32)
            a = jnp.maximum(a, 0).astype(BF16)
            return acc + jnp.dot(a, w2_ref[c * FCH:(c + 1) * FCH, :], preferred_element_type=F32)

        h0, hn0 = wo_part(0, pltpu.bitcast(oa_s[...], BF16))
        acc = h0
        pieces = []
        ng = M // 16
        for c in range(NF):
            acc = ffn_chunk(hn0, c, acc)
            if c < NATT:
                for g in range(c * ng // NATT, (c + 1) * ng // NATT):
                    pieces.append(att16(M + 16 * g))
            if c == WO_POS:
                h1, hn1 = wo_part(1, pltpu.bitcast(jnp.concatenate(pieces, axis=0), BF16))
        o_ref[0:M, :] = acc.astype(o_ref.dtype)
        acc = h1
        for c in range(NF):
            acc = ffn_chunk(hn1, c, acc)
        o_ref[M:2 * M, :] = acc.astype(o_ref.dtype)


@jax.jit
def pallas_sequential_preLN__sliding_local_dilated__dense_activation_relu__prompt_kernel(
    A_x: jax.Array,
    A_wqkv: jax.Array,
    A_wo: jax.Array,
    B_x: jax.Array,
    B_w1: jax.Array,
    B_w2: jax.Array,
):
    x = A_x.reshape(S, D)
    anyspec = pl.BlockSpec(memory_space=pl.ANY)
    out = pl.pallas_call(
        _kernel,
        grid=(2 * NT,),
        in_specs=[pl.BlockSpec((TM, D), lambda i: (i % NT, 0)), anyspec, anyspec, anyspec, anyspec],
        out_specs=pl.BlockSpec((TM, D), lambda i: (jnp.maximum(i - NT, 0), 0)),
        out_shape=jax.ShapeDtypeStruct((S, D), BF16),
        scratch_shapes=[
            pltpu.VMEM((D, 3 * D), BF16),
            pltpu.VMEM((D, D), BF16),
            pltpu.VMEM((D, DFF), BF16),
            pltpu.VMEM((DFF, D), BF16),
            pltpu.SemaphoreType.DMA((6,)),
            pltpu.VMEM((8, S, 128), F32),
            pltpu.VMEM((8, S + HAL, 128), F32),
            pltpu.VMEM((8, S + HAL, 128), F32),
            pltpu.VMEM((S // 4, D), U32),
        ],
        compiler_params=pltpu.CompilerParams(
            dimension_semantics=("arbitrary",), vmem_limit_bytes=100 * 1024 * 1024),
    )(x, A_wqkv, A_wo, B_w1, B_w2)
    return out.reshape(1, S, D)
```

```python
import contextlib
import functools

import jax
import jax.numpy as jnp
import jax.experimental.pallas as pl
import jax.experimental.pallas.tpu as pltpu

S, D, DFF = 2048, 1024, 3584
H, DH, W = 32, 32, 8
I32, U32, F32, BF16 = jnp.int32, jnp.uint32, jnp.float32, jnp.bfloat16
HAL = 16
LOG2E = 1.4426950408889634
TM = 256
M = TM // 2
NT = S // TM
C2 = DH ** -0.5 * LOG2E
EV = {'XLA_TPU_EVENLY_DISTRIBUTE_CRITICAL_NODES': True}


def lane_iota(shape):
    return jax.lax.broadcasted_iota(I32, shape, len(shape) - 1)


def sel_stage(tiles):
    p = (lane_iota(tiles[0].shape) >> 2) & 7
    l0 = [[jnp.where(((p + v) & 1) == 1, tiles[2 * i + 1], tiles[2 * i]) for i in range(4)] for v in range(2)]
    l1 = [[jnp.where((((p + v) >> 1) & 1) == 1, l0[v & 1][2 * i + 1], l0[v & 1][2 * i]) for i in range(2)] for v in range(4)]
    return [jnp.where((((p + j) >> 2) & 1) == 1, l1[j & 3][1], l1[j & 3][0]) for j in range(8)]


def seg_rot(x, sh):
    sh %= 32
    if sh == 0:
        return x
    lane = lane_iota(x.shape)
    idx = (lane & ~31) | ((lane - sh) & 31)
    if x.dtype == U32:
        return jnp.take_along_axis(x.astype(I32), idx, axis=1).astype(U32)
    return jnp.take_along_axis(x, idx, axis=1)


def perm_fwd(tiles):
    n = sel_stage(tiles)
    return [seg_rot(n[j], 4 * j) for j in range(8)]


def perm_inv(tiles):
    n = [seg_rot(tiles[j], -4 * j) for j in range(8)]
    f = (lane_iota(tiles[0].shape) >> 2) & 7
    q = (8 - f) & 7
    l0 = [[jnp.where(((q + v) & 1) == 1, n[2 * i + 1], n[2 * i]) for i in range(4)] for v in range(2)]
    l1 = [[jnp.where((((q + v) >> 1) & 1) == 1, l0[v & 1][2 * i + 1], l0[v & 1][2 * i]) for i in range(2)] for v in range(4)]
    return [jnp.where((((q + t) >> 2) & 1) == 1, l1[t & 3][1], l1[t & 3][0]) for t in range(8)]


def allreduce4(x):
    lane = lane_iota(x.shape)
    y = x + jnp.take_along_axis(x, lane ^ 1, axis=1)
    return y + jnp.take_along_axis(y, lane ^ 2, axis=1)


def ln(x):
    m = jnp.mean(x, axis=-1, keepdims=True)
    xc = x - m
    v = jnp.mean(xc * xc, axis=-1, keepdims=True)
    return xc * jax.lax.rsqrt(v + 1e-5)


def make(fch=896, flags=None, scopes=False, g_nch=4, pk=False, NP1=4, unroll_f=True, osplit=2):
    nf = DFF // fch
    scope = (lambda n: jax.named_scope(n)) if scopes else (lambda n: contextlib.nullcontext())
    R1 = (S - TM) // NP1
    M1 = R1 // 2
    NPRE = 16 // NP1
    assert R1 * NP1 == S - TM and M1 % 16 == 0 and NPRE * NP1 == 16

    def kern(x_hbm, wqkv_hbm, wo_hbm, w1_hbm, w2_hbm, o_hbm,
             x_all, wqkv_in, wqkv_ref, wo_ref, w1_ref, w2_ref, wsems, sems, xsems, osems,
             qkv_all, oa_s, xn_s, xn0_s, qkv0_s, out_s):
        x_first = pltpu.make_async_copy(x_hbm.at[pl.ds(0, TM), :], x_all.at[pl.ds(0, TM), :], xsems.at[0])
        x_mid = pltpu.make_async_copy(x_hbm.at[pl.ds(TM, R1 + M1), :], x_all.at[pl.ds(TM, R1 + M1), :], xsems.at[1])
        x_rest = pltpu.make_async_copy(x_hbm.at[pl.ds(TM + R1 + M1, S - TM - R1 - M1), :],
                                       x_all.at[pl.ds(TM + R1 + M1, S - TM - R1 - M1), :], xsems.at[2])

        def wq_copy(c):
            c0 = c * D if isinstance(c, int) else pl.multiple_of(c * D, D)
            return pltpu.make_async_copy(wqkv_hbm.at[:, pl.ds(c0, D)], wqkv_in.at[c], wsems.at[c])
        if pk:
            wo_p, w1_p, w2_p = wo_hbm.bitcast(U32), w1_hbm.bitcast(U32), w2_hbm.bitcast(U32)
        else:
            wo_p, w1_p, w2_p = wo_hbm, w1_hbm, w2_hbm
        cr = [pltpu.make_async_copy(wo_p, wo_ref, sems.at[0]),
              pltpu.make_async_copy(w1_p, w1_ref, sems.at[1]),
              pltpu.make_async_copy(w2_p, w2_ref, sems.at[2])]

        def ln_rows(r, n):
            x = x_all[pl.ds(r, n), :].astype(F32)
            return ln(x).astype(BF16)

        def wld(ref, r0, r1, c0, c1):
            if not pk:
                return ref[r0:r1, c0:c1]
            return pltpu.bitcast(ref[r0 // 2:r1 // 2, c0:c1], BF16)

        def att_rows(base, n, src, masked):
            q_s = src.at[0, :, pl.ds(base + HAL, n), :]
            k_s = src.at[1, :, pl.ds(base, n + HAL), :]
            v_s = src.at[2, :, pl.ds(base, n + HAL), :]

            def att8(r):
                q = [q_s[j, r:r + 8, :] for j in range(8)]
                t = []
                for w in range(W):
                    acc = functools.reduce(jnp.add, [q[j] * k_s[j, HAL + r - 2 * w:HAL + r - 2 * w + 8, :] for j in range(8)])
                    l = allreduce4(acc) * C2
                    if masked and r < 16 and 2 * w > r:
                        pos = base + r + jax.lax.broadcasted_iota(I32, (8, 128), 0)
                        l = jnp.where(pos >= 2 * w, l, -1e9 * LOG2E)
                    t.append(l)
                m = functools.reduce(jnp.maximum, t)
                e = [jnp.exp2(x - m) for x in t]
                inv = 1.0 / functools.reduce(jnp.add, e)
                a = [x * inv for x in e]
                return [functools.reduce(jnp.add, [a[w] * v_s[j, HAL + r - 2 * w:HAL + r - 2 * w + 8, :] for w in range(W)]) for j in range(8)]

            def att16(g):
                lo, hi = att8(16 * g), att8(16 * g + 8)
                pkd = [pltpu.bitcast(jnp.concatenate([lo[j], hi[j]], axis=0).astype(BF16), U32) for j in range(8)]
                return jnp.concatenate(perm_inv(pkd), axis=1)
            return att16

        with scope("init"):
            x_first.start()
            wq_copy(0).start()
            qkv0_s[1, :, 0:HAL, :] = jnp.zeros((8, HAL, 128), F32)
            qkv0_s[2, :, 0:HAL, :] = jnp.zeros((8, HAL, 128), F32)
            x_first.wait()
            xn0_s[0:M // 2, :] = pltpu.bitcast(ln_rows(0, M), U32)
            xn0_s[M // 2:M, :] = pltpu.bitcast(ln_rows(M, M), U32)

        def g_step(c, _):
          with scope("G"):
            wq_copy(c).wait()
            @pl.when(c < 2)
            def _():
                wq_copy(c + 1).start()
            @pl.when(c == 1)
            def _():
                x_mid.start()
            xn0 = pltpu.bitcast(xn0_s[...], BF16)
            ng = D // 16
            kc = D // g_nch
            y = None
            for n in range(g_nch):
                for g in range(n * ng // g_nch, (n + 1) * ng // g_nch):
                    w = pltpu.bitcast(wqkv_in[c, 16 * g:16 * g + 16, :], U32)
                    tiles = perm_fwd([w[:, t * 128:(t + 1) * 128] for t in range(8)])
                    wqkv_ref[c, 8 * g:8 * g + 8, :] = jnp.concatenate(tiles, axis=1)
                wk = pltpu.bitcast(wqkv_ref[c, n * kc // 2:(n + 1) * kc // 2, :], BF16)
                d = jnp.dot(xn0[:, n * kc:(n + 1) * kc], wk, preferred_element_type=F32)
                y = d if y is None else y + d
            for j in range(8):
                qkv_all[c, j, TM:HAL + TM, :] = y[TM - HAL:TM, j * 128:(j + 1) * 128]
                qkv0_s[c, j, HAL:HAL + TM, :] = y[:, j * 128:(j + 1) * 128]
          return 0
        jax.lax.fori_loop(0, 3, g_step, 0)

        with scope("mid"):
            x_mid.wait()
            x_rest.start()
            xn_s[...] = pltpu.bitcast(ln_rows(TM, M1), U32)

        def p1_step(i, _):
          with scope("P1"):
            @pl.when(i == 1)
            def _():
                x_rest.wait()
                for c in cr:
                    c.start()
            row0 = pl.multiple_of(TM + i * R1, 16)
            gb = pl.multiple_of(i * 16 * NPRE, 16)
            attp = att_rows(gb, 16 * NPRE, qkv0_s, True)
            for g in range(NPRE):
                oa_s[pl.ds(pl.multiple_of(i * 8 * NPRE + 8 * g, 8), 8), :] = attp(g)
            dsts = [qkv_all.at[c, :, pl.ds(row0 + HAL, R1), :] for c in range(3)]
            xa = pltpu.bitcast(xn_s[...], BF16)
            xb = ln_rows(row0 + M1, M1)
            for c in range(3):
                y = jnp.dot(xa, pltpu.bitcast(wqkv_ref[c], BF16), preferred_element_type=F32)
                for j in range(8):
                    dsts[c][j, 0:M1, :] = y[:, j * 128:(j + 1) * 128]
            rn = pl.multiple_of(jnp.minimum(row0 + R1, S - M1), 16)
            xnext = ln_rows(rn, M1)
            for c in range(3):
                y = jnp.dot(xb, pltpu.bitcast(wqkv_ref[c], BF16), preferred_element_type=F32)
                for j in range(8):
                    dsts[c][j, M1:R1, :] = y[:, j * 128:(j + 1) * 128]
            xn_s[...] = pltpu.bitcast(xnext, U32)
          return 0
        jax.lax.fori_loop(0, NP1, p1_step, 0)

        with scope("wait2"):
            for c in cr:
                c.wait()

        OS = TM // osplit
        def o_copy(t, part):
            slot = t % 2
            r = t * TM + part * OS
            r = r if isinstance(t, int) else pl.multiple_of(r, OS)
            return pltpu.make_async_copy(out_s.at[slot, pl.ds(part * OS, OS), :], o_hbm.at[pl.ds(r, OS), :], osems.at[slot, part])

        def p2_step(t, _):
          with scope("P2"):
            row0 = pl.multiple_of(t * TM, TM)
            slot = t % 2

            @pl.when(t >= 2)
            def _():
                for part in range(osplit):
                    o_copy(t - 2, part).wait()

            def wo_part(r, n, o):
                h = x_all[pl.ds(pl.multiple_of(row0 + r, 16), n), :].astype(F32) + jnp.dot(o, wld(wo_ref, 0, D, 0, D), preferred_element_type=F32)
                return h, ln(h).astype(BF16)

            def ffn(hn, acc):
                for c in range(nf):
                    a = jnp.dot(hn, wld(w1_ref, 0, D, c * fch, (c + 1) * fch), preferred_element_type=F32)
                    a = jnp.maximum(a, 0).astype(BF16)
                    acc = acc + jnp.dot(a, wld(w2_ref, c * fch, (c + 1) * fch, 0, D), preferred_element_type=F32)
                return acc

            oa = pltpu.bitcast(oa_s[...], BF16)
            h0, hn0 = wo_part(0, M, oa[0:M])
            h1, hn1 = wo_part(M, M, oa[M:2 * M])
            nxt = pl.multiple_of(jnp.minimum(row0 + TM, S - TM), TM)
            att = att_rows(nxt, TM, qkv_all, False)
            for g in range(16):
                oa_s[8 * g:8 * g + 8, :] = att(g)
            acc = ffn(hn0, h0)
            out_s[slot, 0:M, :] = acc.astype(BF16)
            if osplit == 2:
                o_copy(t, 0).start()
            acc = ffn(hn1, h1)
            out_s[slot, M:2 * M, :] = acc.astype(BF16)
            if osplit == 2:
                o_copy(t, 1).start()
            else:
                o_copy(t, 0).start()
          return 0
        jax.lax.fori_loop(0, NT, p2_step, 0)
        for t in (NT - 2, NT - 1):
            for part in range(osplit):
                o_copy(t, part).wait()

    def fn(A_x, A_wqkv, A_wo, B_x, B_w1, B_w2):
        x = A_x.reshape(S, D)
        anyspec = pl.BlockSpec(memory_space=pl.ANY)
        out = pl.pallas_call(
            kern,
            in_specs=[anyspec, anyspec, anyspec, anyspec, anyspec],
            out_specs=anyspec,
            out_shape=jax.ShapeDtypeStruct((S, D), BF16),
            scratch_shapes=[
                pltpu.VMEM((S, D), BF16),
                pltpu.VMEM((3, D, D), BF16),
                pltpu.VMEM((3, D // 2, D), U32),
                pltpu.VMEM((D // 2, D), U32) if pk else pltpu.VMEM((D, D), BF16),
                pltpu.VMEM((D // 2, DFF), U32) if pk else pltpu.VMEM((D, DFF), BF16),
                pltpu.VMEM((DFF // 2, D), U32) if pk else pltpu.VMEM((DFF, D), BF16),
                pltpu.SemaphoreType.DMA((3,)),
                pltpu.SemaphoreType.DMA((3,)),
                pltpu.SemaphoreType.DMA((3,)),
                pltpu.SemaphoreType.DMA((2, osplit)),
                pltpu.VMEM((3, 8, S + HAL, 128), F32),
                pltpu.VMEM((M, D), U32),
                pltpu.VMEM((M1 // 2, D), U32),
                pltpu.VMEM((M, D), U32),
                pltpu.VMEM((3, 8, TM + HAL, 128), F32),
                pltpu.VMEM((2, TM, D), BF16),
            ],
            compiler_params=pltpu.CompilerParams(vmem_limit_bytes=110 * 1024 * 1024, flags=flags),
        )(x, A_wqkv, A_wo, B_w1, B_w2)
        return out.reshape(1, S, D)
    return fn


_impl = make(g_nch=8)


@jax.jit
def pallas_sequential_preLN__sliding_local_dilated__dense_activation_relu__prompt_kernel(
    A_x: jax.Array,
    A_wqkv: jax.Array,
    A_wo: jax.Array,
    B_x: jax.Array,
    B_w1: jax.Array,
    B_w2: jax.Array,
):
    return _impl(A_x, A_wqkv, A_wo, B_x, B_w1, B_w2)
```

```python
import contextlib
import functools

import jax
import jax.numpy as jnp
import jax.experimental.pallas as pl
import jax.experimental.pallas.tpu as pltpu

S, D, DFF = 2048, 1024, 3584
H, DH, W = 32, 32, 8
I32, U32, F32, BF16 = jnp.int32, jnp.uint32, jnp.float32, jnp.bfloat16
HAL = 16
LOG2E = 1.4426950408889634
TM = 256
M = TM // 2
NT = S // TM
C2 = DH ** -0.5 * LOG2E
EV = {'XLA_TPU_EVENLY_DISTRIBUTE_CRITICAL_NODES': True}


def lane_iota(shape):
    return jax.lax.broadcasted_iota(I32, shape, len(shape) - 1)


def sel_stage(tiles):
    p = (lane_iota(tiles[0].shape) >> 2) & 7
    l0 = [[jnp.where(((p + v) & 1) == 1, tiles[2 * i + 1], tiles[2 * i]) for i in range(4)] for v in range(2)]
    l1 = [[jnp.where((((p + v) >> 1) & 1) == 1, l0[v & 1][2 * i + 1], l0[v & 1][2 * i]) for i in range(2)] for v in range(4)]
    return [jnp.where((((p + j) >> 2) & 1) == 1, l1[j & 3][1], l1[j & 3][0]) for j in range(8)]


def seg_rot(x, sh):
    sh %= 32
    if sh == 0:
        return x
    lane = lane_iota(x.shape)
    idx = (lane & ~31) | ((lane - sh) & 31)
    if x.dtype == U32:
        return jnp.take_along_axis(x.astype(I32), idx, axis=1).astype(U32)
    return jnp.take_along_axis(x, idx, axis=1)


def perm_fwd(tiles):
    n = sel_stage(tiles)
    return [seg_rot(n[j], 4 * j) for j in range(8)]


def perm_inv(tiles):
    n = [seg_rot(tiles[j], -4 * j) for j in range(8)]
    f = (lane_iota(tiles[0].shape) >> 2) & 7
    q = (8 - f) & 7
    l0 = [[jnp.where(((q + v) & 1) == 1, n[2 * i + 1], n[2 * i]) for i in range(4)] for v in range(2)]
    l1 = [[jnp.where((((q + v) >> 1) & 1) == 1, l0[v & 1][2 * i + 1], l0[v & 1][2 * i]) for i in range(2)] for v in range(4)]
    return [jnp.where((((q + t) >> 2) & 1) == 1, l1[t & 3][1], l1[t & 3][0]) for t in range(8)]


def allreduce4(x):
    lane = lane_iota(x.shape)
    y = x + jnp.take_along_axis(x, lane ^ 1, axis=1)
    return y + jnp.take_along_axis(y, lane ^ 2, axis=1)


def ln(x):
    m = jnp.mean(x, axis=-1, keepdims=True)
    xc = x - m
    v = jnp.mean(xc * xc, axis=-1, keepdims=True)
    return xc * jax.lax.rsqrt(v + 1e-5)


def make(fch=896, flags=None, scopes=False, g_nch=4, pk=False, NP1=4, unroll_f=True, osplit=2, attpos=0, p1attpos=0, p1order=0, lnpos=0, late_out=False, wsplit=1, xafter=False):
    nf = DFF // fch
    scope = (lambda n: jax.named_scope(n)) if scopes else (lambda n: contextlib.nullcontext())
    R1 = (S - TM) // NP1
    M1 = R1 // 2
    NPRE = 16 // NP1
    assert R1 * NP1 == S - TM and M1 % 16 == 0 and NPRE * NP1 == 16

    def kern(x_hbm, wqkv_hbm, wo_hbm, w1_hbm, w2_hbm, o_hbm,
             x_all, wqkv_in, wqkv_ref, wo_ref, w1_ref, w2_ref, wsems, sems, xsems, osems,
             qkv_all, oa_s, xn_s, xn0_s, qkv0_s, out_s):
        x_first = pltpu.make_async_copy(x_hbm.at[pl.ds(0, TM), :], x_all.at[pl.ds(0, TM), :], xsems.at[0])
        x_mid = pltpu.make_async_copy(x_hbm.at[pl.ds(TM, R1 + M1), :], x_all.at[pl.ds(TM, R1 + M1), :], xsems.at[1])
        x_rest = pltpu.make_async_copy(x_hbm.at[pl.ds(TM + R1 + M1, S - TM - R1 - M1), :],
                                       x_all.at[pl.ds(TM + R1 + M1, S - TM - R1 - M1), :], xsems.at[2])

        def wq_copy(c):
            c0 = c * D if isinstance(c, int) else pl.multiple_of(c * D, D)
            if wsplit == 1:
                return pltpu.make_async_copy(wqkv_hbm.at[:, pl.ds(c0, D)], wqkv_in.at[c], wsems.at[c])
            rows = D // wsplit
            cps = [pltpu.make_async_copy(wqkv_hbm.at[pl.ds(p * rows, rows), pl.ds(c0, D)], wqkv_in.at[c, pl.ds(p * rows, rows), :], wsems.at[c]) for p in range(wsplit)]
            class Multi:
                def start(self_):
                    for cp in cps: cp.start()
                def wait(self_):
                    for cp in cps: cp.wait()
            return Multi()
        if pk:
            wo_p, w1_p, w2_p = wo_hbm.bitcast(U32), w1_hbm.bitcast(U32), w2_hbm.bitcast(U32)
        else:
            wo_p, w1_p, w2_p = wo_hbm, w1_hbm, w2_hbm
        cr = [pltpu.make_async_copy(wo_p, wo_ref, sems.at[0]),
              pltpu.make_async_copy(w1_p, w1_ref, sems.at[1]),
              pltpu.make_async_copy(w2_p, w2_ref, sems.at[2])]

        def ln_rows(r, n):
            x = x_all[pl.ds(r, n), :].astype(F32)
            return ln(x).astype(BF16)

        def wld(ref, r0, r1, c0, c1):
            if not pk:
                return ref[r0:r1, c0:c1]
            return pltpu.bitcast(ref[r0 // 2:r1 // 2, c0:c1], BF16)

        def att_rows(base, n, src, masked):
            q_s = src.at[0, :, pl.ds(base + HAL, n), :]
            k_s = src.at[1, :, pl.ds(base, n + HAL), :]
            v_s = src.at[2, :, pl.ds(base, n + HAL), :]

            def att8(r):
                q = [q_s[j, r:r + 8, :] for j in range(8)]
                t = []
                for w in range(W):
                    acc = functools.reduce(jnp.add, [q[j] * k_s[j, HAL + r - 2 * w:HAL + r - 2 * w + 8, :] for j in range(8)])
                    l = allreduce4(acc) * C2
                    if masked and r < 16 and 2 * w > r:
                        pos = base + r + jax.lax.broadcasted_iota(I32, (8, 128), 0)
                        l = jnp.where(pos >= 2 * w, l, -1e9 * LOG2E)
                    t.append(l)
                m = functools.reduce(jnp.maximum, t)
                e = [jnp.exp2(x - m) for x in t]
                inv = 1.0 / functools.reduce(jnp.add, e)
                a = [x * inv for x in e]
                return [functools.reduce(jnp.add, [a[w] * v_s[j, HAL + r - 2 * w:HAL + r - 2 * w + 8, :] for w in range(W)]) for j in range(8)]

            def att16(g):
                lo, hi = att8(16 * g), att8(16 * g + 8)
                pkd = [pltpu.bitcast(jnp.concatenate([lo[j], hi[j]], axis=0).astype(BF16), U32) for j in range(8)]
                return jnp.concatenate(perm_inv(pkd), axis=1)
            return att16

        with scope("init"):
            if xafter:
                wq_copy(0).start()
                x_first.start()
            else:
                x_first.start()
                wq_copy(0).start()
            x_first.wait()
            xn0_s[0:M // 2, :] = pltpu.bitcast(ln_rows(0, M), U32)
            xn0_s[M // 2:M, :] = pltpu.bitcast(ln_rows(M, M), U32)

        def g_step(c, _):
          with scope("G"):
            wq_copy(c).wait()
            @pl.when(c < 2)
            def _():
                wq_copy(c + 1).start()
            @pl.when(c == 1)
            def _():
                x_mid.start()
            xn0 = pltpu.bitcast(xn0_s[...], BF16)
            ng = D // 16
            kc = D // g_nch
            y = None
            for n in range(g_nch):
                for g in range(n * ng // g_nch, (n + 1) * ng // g_nch):
                    w = pltpu.bitcast(wqkv_in[c, 16 * g:16 * g + 16, :], U32)
                    tiles = perm_fwd([w[:, t * 128:(t + 1) * 128] for t in range(8)])
                    wqkv_ref[c, 8 * g:8 * g + 8, :] = jnp.concatenate(tiles, axis=1)
                wk = pltpu.bitcast(wqkv_ref[c, n * kc // 2:(n + 1) * kc // 2, :], BF16)
                d = jnp.dot(xn0[:, n * kc:(n + 1) * kc], wk, preferred_element_type=F32)
                y = d if y is None else y + d
            for j in range(8):
                qkv_all[c, j, TM:HAL + TM, :] = y[TM - HAL:TM, j * 128:(j + 1) * 128]
                qkv0_s[c, j, HAL:HAL + TM, :] = y[:, j * 128:(j + 1) * 128]
                qkv0_s[c, j, 0:HAL, :] = jnp.broadcast_to(y[0:1, j * 128:(j + 1) * 128], (HAL, 128))
          return 0
        jax.lax.fori_loop(0, 3, g_step, 0)

        with scope("mid"):
            x_mid.wait()
            x_rest.start()
            xn_s[...] = pltpu.bitcast(ln_rows(TM, M1), U32)

        def p1_step(i, _):
          with scope("P1"):
            @pl.when(i == 1)
            def _():
                x_rest.wait()
                for c in cr:
                    c.start()
            row0 = pl.multiple_of(TM + i * R1, 16)
            gb = pl.multiple_of(i * 16 * NPRE, 16)
            attp = att_rows(gb, 16 * NPRE, qkv0_s, True)
            def do_attp():
                for g in range(NPRE):
                    oa_s[pl.ds(pl.multiple_of(i * 8 * NPRE + 8 * g, 8), 8), :] = attp(g)
            if p1attpos == 0:
                do_attp()
            dsts = [qkv_all.at[c, :, pl.ds(row0 + HAL, R1), :] for c in range(3)]
            xa = pltpu.bitcast(xn_s[...], BF16)
            xb = ln_rows(row0 + M1, M1)
            rn = pl.multiple_of(jnp.minimum(row0 + R1, S - M1), 16)
            if lnpos == 1:
                xnext = ln_rows(rn, M1)
                xn_s[...] = pltpu.bitcast(xnext, U32)
            def part(xx, r0, c):
                y = jnp.dot(xx, pltpu.bitcast(wqkv_ref[c], BF16), preferred_element_type=F32)
                for j in range(8):
                    dsts[c][j, r0:r0 + M1, :] = y[:, j * 128:(j + 1) * 128]
            if p1order == 0:
                for c in range(3):
                    part(xa, 0, c)
                if p1attpos == 1:
                    do_attp()
                if lnpos == 0:
                    xnext = ln_rows(rn, M1)
                for c in range(3):
                    part(xb, M1, c)
            else:
                part(xa, 0, 0)
                part(xa, 0, 1)
                part(xb, M1, 0)
                if p1attpos == 1:
                    do_attp()
                if lnpos == 0:
                    xnext = ln_rows(rn, M1)
                part(xb, M1, 1)
                part(xa, 0, 2)
                part(xb, M1, 2)
            if p1attpos == 2:
                do_attp()
            if lnpos == 0:
                xn_s[...] = pltpu.bitcast(xnext, U32)
          return 0
        jax.lax.fori_loop(0, NP1, p1_step, 0)

        with scope("wait2"):
            for c in cr:
                c.wait()

        OS = TM // osplit
        def o_copy(t, part):
            slot = t % 2
            r = t * TM + part * OS
            r = r if isinstance(t, int) else pl.multiple_of(r, OS)
            return pltpu.make_async_copy(out_s.at[slot, pl.ds(part * OS, OS), :], o_hbm.at[pl.ds(r, OS), :], osems.at[slot, part])

        def p2_step(t, _):
          with scope("P2"):
            row0 = pl.multiple_of(t * TM, TM)
            slot = t % 2

            if late_out:
                @pl.when(t >= 1)
                def _():
                    o_copy(t - 1, 1).start()
            @pl.when(t >= 2)
            def _():
                for part in range(osplit):
                    o_copy(t - 2, part).wait()

            def wo_part(r, n, o):
                h = x_all[pl.ds(pl.multiple_of(row0 + r, 16), n), :].astype(F32) + jnp.dot(o, wld(wo_ref, 0, D, 0, D), preferred_element_type=F32)
                return h, ln(h).astype(BF16)

            def ffn(hn, acc):
                for c in range(nf):
                    a = jnp.dot(hn, wld(w1_ref, 0, D, c * fch, (c + 1) * fch), preferred_element_type=F32)
                    a = jnp.maximum(a, 0).astype(BF16)
                    acc = acc + jnp.dot(a, wld(w2_ref, c * fch, (c + 1) * fch, 0, D), preferred_element_type=F32)
                return acc

            oa = pltpu.bitcast(oa_s[...], BF16)
            h0, hn0 = wo_part(0, M, oa[0:M])
            h1, hn1 = wo_part(M, M, oa[M:2 * M])
            nxt = pl.multiple_of(jnp.minimum(row0 + TM, S - TM), TM)
            att = att_rows(nxt, TM, qkv_all, False)
            def do_att(g0, g1):
                for g in range(g0, g1):
                    oa_s[8 * g:8 * g + 8, :] = att(g)
            if attpos == 0:
                do_att(0, 16)
            elif attpos == 1:
                do_att(0, 8)
            acc = ffn(hn0, h0)
            out_s[slot, 0:M, :] = acc.astype(BF16)
            if osplit == 2:
                o_copy(t, 0).start()
            if attpos == 1:
                do_att(8, 16)
            elif attpos == 2:
                do_att(0, 16)
            acc = ffn(hn1, h1)
            out_s[slot, M:2 * M, :] = acc.astype(BF16)
            if late_out:
                pass
            elif osplit == 2:
                o_copy(t, 1).start()
            else:
                o_copy(t, 0).start()
          return 0
        jax.lax.fori_loop(0, NT, p2_step, 0)
        if late_out:
            o_copy(NT - 1, 1).start()
        for t in (NT - 2, NT - 1):
            for part in range(osplit):
                o_copy(t, part).wait()

    def fn(A_x, A_wqkv, A_wo, B_x, B_w1, B_w2):
        x = A_x.reshape(S, D)
        anyspec = pl.BlockSpec(memory_space=pl.ANY)
        out = pl.pallas_call(
            kern,
            in_specs=[anyspec, anyspec, anyspec, anyspec, anyspec],
            out_specs=anyspec,
            out_shape=jax.ShapeDtypeStruct((S, D), BF16),
            scratch_shapes=[
                pltpu.VMEM((S, D), BF16),
                pltpu.VMEM((3, D, D), BF16),
                pltpu.VMEM((3, D // 2, D), U32),
                pltpu.VMEM((D // 2, D), U32) if pk else pltpu.VMEM((D, D), BF16),
                pltpu.VMEM((D // 2, DFF), U32) if pk else pltpu.VMEM((D, DFF), BF16),
                pltpu.VMEM((DFF // 2, D), U32) if pk else pltpu.VMEM((DFF, D), BF16),
                pltpu.SemaphoreType.DMA((3,)),
                pltpu.SemaphoreType.DMA((3,)),
                pltpu.SemaphoreType.DMA((3,)),
                pltpu.SemaphoreType.DMA((2, osplit)),
                pltpu.VMEM((3, 8, S + HAL, 128), F32),
                pltpu.VMEM((M, D), U32),
                pltpu.VMEM((M1 // 2, D), U32),
                pltpu.VMEM((M, D), U32),
                pltpu.VMEM((3, 8, TM + HAL, 128), F32),
                pltpu.VMEM((2, TM, D), BF16),
            ],
            compiler_params=pltpu.CompilerParams(vmem_limit_bytes=110 * 1024 * 1024, flags=flags),
        )(x, A_wqkv, A_wo, B_w1, B_w2)
        return out.reshape(1, S, D)
    return fn


_impl = make(g_nch=8)


@jax.jit
def pallas_sequential_preLN__sliding_local_dilated__dense_activation_relu__prompt_kernel(
    A_x: jax.Array,
    A_wqkv: jax.Array,
    A_wo: jax.Array,
    B_x: jax.Array,
    B_w1: jax.Array,
    B_w2: jax.Array,
):
    return _impl(A_x, A_wqkv, A_wo, B_x, B_w1, B_w2)
```

```python
import functools

import jax
import jax.numpy as jnp
import jax.experimental.pallas as pl
import jax.experimental.pallas.tpu as pltpu

S, D, DFF = 2048, 1024, 3584
DH, W = 32, 8
I32, U32, F32, BF16 = jnp.int32, jnp.uint32, jnp.float32, jnp.bfloat16
LOG2E = 1.4426950408889634
C2 = DH ** -0.5 * LOG2E
HAL = 16

TM = 256
M = TM // 2
NT = S // TM
FCH = 896
NF = DFF // FCH
T0 = 288
NP1 = 5
R1 = (S - T0) // NP1
M1 = R1 // 2
NPRE = -(-16 // NP1)
GCH = 8
assert R1 * NP1 == S - T0 and M1 % 16 == 0 and T0 % 32 == 0 and T0 >= TM


def _lane_iota(shape):
    return jax.lax.broadcasted_iota(I32, shape, len(shape) - 1)


def _select8(tiles, idx):
    l0 = [[jnp.where(((idx + v) & 1) == 1, tiles[2 * i + 1], tiles[2 * i]) for i in range(4)]
          for v in range(2)]
    l1 = [[jnp.where((((idx + v) >> 1) & 1) == 1, l0[v & 1][2 * i + 1], l0[v & 1][2 * i])
           for i in range(2)] for v in range(4)]
    return [jnp.where((((idx + j) >> 2) & 1) == 1, l1[j & 3][1], l1[j & 3][0]) for j in range(8)]


def _seg_rot(x, sh):
    sh %= 32
    if sh == 0:
        return x
    lane = _lane_iota(x.shape)
    idx = (lane & ~31) | ((lane - sh) & 31)
    return jnp.take_along_axis(x.astype(I32), idx, axis=1).astype(U32)


def _perm_fwd(tiles):
    n = _select8(tiles, (_lane_iota(tiles[0].shape) >> 2) & 7)
    return [_seg_rot(n[j], 4 * j) for j in range(8)]


def _perm_inv(tiles):
    n = [_seg_rot(tiles[j], -4 * j) for j in range(8)]
    f = (_lane_iota(tiles[0].shape) >> 2) & 7
    return _select8(n, (8 - f) & 7)


def _allreduce4(x):
    lane = _lane_iota(x.shape)
    y = x + jnp.take_along_axis(x, lane ^ 1, axis=1)
    return y + jnp.take_along_axis(y, lane ^ 2, axis=1)


def _ln(x):
    m = jnp.mean(x, axis=-1, keepdims=True)
    xc = x - m
    v = jnp.mean(xc * xc, axis=-1, keepdims=True)
    return xc * jax.lax.rsqrt(v + 1e-5)


def _attention(src, base, n, masked):
    q_s = src.at[0, :, pl.ds(base + HAL, n), :]
    k_s = src.at[1, :, pl.ds(base, n + HAL), :]
    v_s = src.at[2, :, pl.ds(base, n + HAL), :]

    def att8(r):
        q = [q_s[j, r:r + 8, :] for j in range(8)]
        t = []
        for w in range(W):
            acc = functools.reduce(
                jnp.add, [q[j] * k_s[j, HAL + r - 2 * w:HAL + r - 2 * w + 8, :] for j in range(8)])
            l = _allreduce4(acc) * C2
            if masked and r < 16 and 2 * w > r:
                pos = base + r + jax.lax.broadcasted_iota(I32, (8, 128), 0)
                l = jnp.where(pos >= 2 * w, l, -1e9 * LOG2E)
            t.append(l)
        m = functools.reduce(jnp.maximum, t)
        e = [jnp.exp2(x - m) for x in t]
        inv = 1.0 / functools.reduce(jnp.add, e)
        a = [x * inv for x in e]
        return [functools.reduce(
            jnp.add, [a[w] * v_s[j, HAL + r - 2 * w:HAL + r - 2 * w + 8, :] for w in range(W)])
            for j in range(8)]

    def att16(g):
        lo, hi = att8(16 * g), att8(16 * g + 8)
        packed = [pltpu.bitcast(jnp.concatenate([lo[j], hi[j]], axis=0).astype(BF16), U32)
                  for j in range(8)]
        return jnp.concatenate(_perm_inv(packed), axis=1)

    return att16


def _kernel(x_hbm, wqkv_hbm, wo_hbm, w1_hbm, w2_hbm, o_hbm,
            x_all, wqkv_in, wqkv_ref, wo_ref, w1_ref, w2_ref, wsems, sems, xsems, osems,
            qkv_all, oa_s, xn_s, xn0_s, qkv0_s, out_s):
    xa0, xa1 = T0, T0 + R1 + M1
    x_first = pltpu.make_async_copy(
        x_hbm.at[pl.ds(0, xa0), :], x_all.at[pl.ds(0, xa0), :], xsems.at[0])
    x_mid = pltpu.make_async_copy(
        x_hbm.at[pl.ds(xa0, xa1 - xa0), :], x_all.at[pl.ds(xa0, xa1 - xa0), :], xsems.at[1])
    x_rest = pltpu.make_async_copy(
        x_hbm.at[pl.ds(xa1, S - xa1), :], x_all.at[pl.ds(xa1, S - xa1), :], xsems.at[2])

    def wq_copy(c):
        c0 = c * D if isinstance(c, int) else pl.multiple_of(c * D, D)
        return pltpu.make_async_copy(wqkv_hbm.at[:, pl.ds(c0, D)], wqkv_in.at[c], wsems.at[c])

    rest_copies = [pltpu.make_async_copy(wo_hbm, wo_ref, sems.at[0]),
                   pltpu.make_async_copy(w1_hbm, w1_ref, sems.at[1]),
                   pltpu.make_async_copy(w2_hbm, w2_ref, sems.at[2])]

    def ln_rows(r, n):
        return _ln(x_all[pl.ds(r, n), :].astype(F32)).astype(BF16)

    x_first.start()
    wq_copy(0).start()
    x_first.wait()
    xn0_s[0:T0 // 4, :] = pltpu.bitcast(ln_rows(0, T0 // 2), U32)
    xn0_s[T0 // 4:T0 // 2, :] = pltpu.bitcast(ln_rows(T0 // 2, T0 // 2), U32)

    def g_step(c, _):
        wq_copy(c).wait()

        @pl.when(c < 2)
        def _():
            wq_copy(c + 1).start()

        @pl.when(c == 1)
        def _():
            x_mid.start()

        xn0 = pltpu.bitcast(xn0_s[...], BF16)
        ng = D // 16
        kc = D // GCH
        y = None
        for n in range(GCH):
            for g in range(n * ng // GCH, (n + 1) * ng // GCH):
                w = pltpu.bitcast(wqkv_in[c, 16 * g:16 * g + 16, :], U32)
                tiles = _perm_fwd([w[:, t * 128:(t + 1) * 128] for t in range(8)])
                wqkv_ref[c, 8 * g:8 * g + 8, :] = jnp.concatenate(tiles, axis=1)
            wk = pltpu.bitcast(wqkv_ref[c, n * kc // 2:(n + 1) * kc // 2, :], BF16)
            d = jnp.dot(xn0[:, n * kc:(n + 1) * kc], wk, preferred_element_type=F32)
            y = d if y is None else y + d
        for j in range(8):
            yj = y[:, j * 128:(j + 1) * 128]
            qkv_all[c, j, TM:HAL + T0, :] = yj[TM - HAL:T0]
            qkv0_s[c, j, HAL:HAL + TM, :] = yj[0:TM]
            qkv0_s[c, j, 0:HAL, :] = jnp.broadcast_to(yj[0:1], (HAL, 128))
        return 0

    jax.lax.fori_loop(0, 3, g_step, 0)

    x_mid.wait()
    x_rest.start()
    xn_s[...] = pltpu.bitcast(ln_rows(T0, M1), U32)

    def p1_step(i, _):
        @pl.when(i == 1)
        def _():
            x_rest.wait()
            for c in rest_copies:
                c.start()

        row0 = pl.multiple_of(T0 + i * R1, 16)
        g0 = jnp.minimum(i * NPRE, 16 - NPRE)
        attp = _attention(qkv0_s, pl.multiple_of(g0 * 16, 16), 16 * NPRE, True)
        for g in range(NPRE):
            oa_s[pl.ds(pl.multiple_of(g0 * 8 + 8 * g, 8), 8), :] = attp(g)
        dsts = [qkv_all.at[c, :, pl.ds(row0 + HAL, R1), :] for c in range(3)]
        xa = pltpu.bitcast(xn_s[...], BF16)
        xb = ln_rows(row0 + M1, M1)
        rn = pl.multiple_of(jnp.minimum(row0 + R1, S - M1), 16)

        def part(xx, r0, c):
            y = jnp.dot(xx, pltpu.bitcast(wqkv_ref[c], BF16), preferred_element_type=F32)
            for j in range(8):
                dsts[c][j, r0:r0 + M1, :] = y[:, j * 128:(j + 1) * 128]

        for c in range(3):
            part(xa, 0, c)
        xnext = ln_rows(rn, M1)
        for c in range(3):
            part(xb, M1, c)
        xn_s[...] = pltpu.bitcast(xnext, U32)
        return 0

    jax.lax.fori_loop(0, NP1, p1_step, 0)

    for c in rest_copies:
        c.wait()

    def o_copy(t, half):
        r = t * TM + half * M
        r = r if isinstance(t, int) else pl.multiple_of(r, M)
        return pltpu.make_async_copy(
            out_s.at[t % 2, pl.ds(half * M, M), :], o_hbm.at[pl.ds(r, M), :], osems.at[t % 2, half])

    def p2_step(t, _):
        row0 = pl.multiple_of(t * TM, TM)
        slot = t % 2

        @pl.when(t >= 2)
        def _():
            for half in range(2):
                o_copy(t - 2, half).wait()

        def wo_part(r, o):
            h = (x_all[pl.ds(pl.multiple_of(row0 + r, 16), M), :].astype(F32)
                 + jnp.dot(o, wo_ref[...], preferred_element_type=F32))
            return h, _ln(h).astype(BF16)

        def ffn(hn, acc):
            for c in range(NF):
                a = jnp.dot(hn, w1_ref[:, c * FCH:(c + 1) * FCH], preferred_element_type=F32)
                a = jnp.maximum(a, 0).astype(BF16)
                acc = acc + jnp.dot(a, w2_ref[c * FCH:(c + 1) * FCH, :], preferred_element_type=F32)
            return acc

        oa = pltpu.bitcast(oa_s[...], BF16)
        h0, hn0 = wo_part(0, oa[0:M])
        h1, hn1 = wo_part(M, oa[M:2 * M])
        nxt = pl.multiple_of(jnp.minimum(row0 + TM, S - TM), TM)
        att = _attention(qkv_all, nxt, TM, False)
        for g in range(16):
            oa_s[8 * g:8 * g + 8, :] = att(g)
        out_s[slot, 0:M, :] = ffn(hn0, h0).astype(BF16)
        o_copy(t, 0).start()
        out_s[slot, M:2 * M, :] = ffn(hn1, h1).astype(BF16)
        o_copy(t, 1).start()
        return 0

    jax.lax.fori_loop(0, NT, p2_step, 0)
    for t in (NT - 2, NT - 1):
        for half in range(2):
            o_copy(t, half).wait()


@jax.jit
def pallas_sequential_preLN__sliding_local_dilated__dense_activation_relu__prompt_kernel(
    A_x: jax.Array,
    A_wqkv: jax.Array,
    A_wo: jax.Array,
    B_x: jax.Array,
    B_w1: jax.Array,
    B_w2: jax.Array,
):
    del B_x
    x = A_x.reshape(S, D)
    hbm = pl.BlockSpec(memory_space=pl.ANY)
    out = pl.pallas_call(
        _kernel,
        in_specs=[hbm, hbm, hbm, hbm, hbm],
        out_specs=hbm,
        out_shape=jax.ShapeDtypeStruct((S, D), BF16),
        scratch_shapes=[
            pltpu.VMEM((S, D), BF16),
            pltpu.VMEM((3, D, D), BF16),
            pltpu.VMEM((3, D // 2, D), U32),
            pltpu.VMEM((D, D), BF16),
            pltpu.VMEM((D, DFF), BF16),
            pltpu.VMEM((DFF, D), BF16),
            pltpu.SemaphoreType.DMA((3,)),
            pltpu.SemaphoreType.DMA((3,)),
            pltpu.SemaphoreType.DMA((3,)),
            pltpu.SemaphoreType.DMA((2, 2)),
            pltpu.VMEM((3, 8, S + HAL, 128), F32),
            pltpu.VMEM((M, D), U32),
            pltpu.VMEM((M1 // 2, D), U32),
            pltpu.VMEM((T0 // 2, D), U32),
            pltpu.VMEM((3, 8, TM + HAL, 128), F32),
            pltpu.VMEM((2, TM, D), BF16),
        ],
        compiler_params=pltpu.CompilerParams(vmem_limit_bytes=110 * 1024 * 1024),
    )(x, A_wqkv, A_wo, B_w1, B_w2)
    return out.reshape(1, S, D)
```
